```python
import jax
import jax.numpy as jnp

def _softmax(x, axis=-1):
    return jax.nn.softmax(x, axis=axis)

def _gelu(x):
    return jax.nn.gelu(x, approximate=True)

def _silu(x):
    return jax.nn.silu(x)

def _sigmoid(x):
    return jax.nn.sigmoid(x)

def _layernorm(x, axis=-1, eps=1e-05):
    m = jnp.mean(x, axis=axis, keepdims=True)
    v = jnp.var(x, axis=axis, keepdims=True)
    return (x - m) / jnp.sqrt(v + eps)

def _scatter_add(tgt, idx, src, axis=0):
    return tgt.at[idx].add(src)

def _segment_sum(src, seg, n):
    return jax.ops.segment_sum(src, seg, n)

class _Rng:

    def __init__(self, key):
        self._k = key

    def _next(self):
        self._k, sub = jax.random.split(self._k)
        return sub

    def normal(self, shape):
        return jax.random.normal(self._next(), shape, dtype=jnp.bfloat16)

    def randint(self, lo, hi, shape):
        return jax.random.randint(self._next(), shape, lo, hi, dtype=jnp.int32)

    def uniform(self, shape, lo=0.0, hi=1.0):
        return jax.random.uniform(self._next(), shape, jnp.bfloat16, lo, hi)

    def permutation(self, n):
        return jax.random.permutation(self._next(), n)
kernel_name = 'adaLN_cond__sliding_block_cached__glu_gated_bilinear__decode'

def setup_inputs():
    _rng = _Rng(jax.random.key(int.from_bytes(__import__("os").urandom(4), "little")))
    _w = lambda a: (lambda t: t.astype(jnp.bfloat16) if jnp.issubdtype(t.dtype, jnp.floating) else t)(jnp.asarray(a))

    def _A_setup():
        B, Sq, D = (1, 1, 640)
        Hq, Hkv, Sk, Dh = (32, 32, 32768, 192)
        assert Hq % Hkv == 0, (Hq, Hkv)
        return {'x': _w((lambda *s: _rng.normal(s) * 0.05)(B, Sq, D)), 'k_cache': _w((lambda *s: _rng.normal(s) * 0.05)(B, Hkv, Sk, Dh)), 'v_cache': _w((lambda *s: _rng.normal(s) * 0.05)(B, Hkv, Sk, Dh)), 'wq': _w((lambda *s: _rng.normal(s) * 0.05)(D, Hq * Dh) * D ** (-0.5)), 'wo': _w((lambda *s: _rng.normal(s) * 0.05)(Hq * Dh, D) * (Hq * Dh) ** (-0.5))}
    _A_in = _A_setup()

    def _B_setup():
        B, S, D, F = (1, 1, 640, 1536)
        return {'x': _w((lambda *s: _rng.normal(s) * 0.05)(B, S, D)), 'w_gate': _w((lambda *s: _rng.normal(s) * 0.05)(D, F) * D ** (-0.5)), 'w_up': _w((lambda *s: _rng.normal(s) * 0.05)(D, F) * D ** (-0.5)), 'w_down': _w((lambda *s: _rng.normal(s) * 0.05)(F, D) * F ** (-0.5))}
    _B_in = _B_setup()
    return {'A_x': _A_in['x'], 'A_k_cache': _A_in['k_cache'], 'A_v_cache': _A_in['v_cache'], 'A_wq': _A_in['wq'], 'A_wo': _A_in['wo'], 'B_x': _B_in['x'], 'B_w_gate': _B_in['w_gate'], 'B_w_up': _B_in['w_up'], 'B_w_down': _B_in['w_down'], 'c': _w((lambda *s: _rng.normal(s) * 0.05)(1, 640)), 'w_mod': _w((lambda *s: _rng.normal(s) * 0.05)(640, 6 * 640) * 640 ** (-0.5))}

def reference(A_x, A_k_cache, A_v_cache, A_wq, A_wo, B_x, B_w_gate, B_w_up, B_w_down, c, w_mod):

    def _A_ref(x, k_cache, v_cache, wq, wo):
        B, Sq, D = x.shape
        Hq, Dh = (32, 192)
        Hkv, Sk = (k_cache.shape[1], k_cache.shape[2])
        W = min(4096, max(256, Sk // 4))
        rep = Hq // Hkv
        q = (lambda x, *d: x.transpose(*d))((x @ wq).reshape(B, Sq, Hq, Dh), 0, 2, 1, 3)
        k = jnp.repeat(k_cache[:, :, Sk - W:, :], rep, axis=1)
        v = jnp.repeat(v_cache[:, :, Sk - W:, :], rep, axis=1)
        scores = jnp.einsum('bhqd,bhkd->bhqk', q, k) * Dh ** (-0.5)
        p = _softmax(scores, axis=-1)
        o = jnp.einsum('bhqk,bhkd->bhqd', p, v)
        return (lambda x, *d: x.transpose(*d))(o, 0, 2, 1, 3).reshape(B, Sq, Hq * Dh) @ wo

    def _B_ref(x, w_gate, w_up, w_down):
        g = jnp.einsum('bsd,df->bsf', x, w_gate)
        u = jnp.einsum('bsd,df->bsf', x, w_up)
        h = g * u
        return jnp.einsum('bsf,fd->bsd', h, w_down)
    x = A_x
    mod = (_silu(c) @ w_mod).reshape(c.shape[0], 6, 1, -1)
    sa, ca, ga, sb, cb, gb = (mod[:, 0].copy(), mod[:, 1].copy(), mod[:, 2].copy(), mod[:, 3].copy(), mod[:, 4].copy(), mod[:, 5].copy())
    h = _layernorm(x, axis=-1) * (1 + ca) + sa
    x = x + ga * _A_ref(h, A_k_cache, A_v_cache, A_wq, A_wo)
    h = _layernorm(x, axis=-1) * (1 + cb) + sb
    x = x + gb * _B_ref(h, B_w_gate, B_w_up, B_w_down)
    return x
```

```python
import functools

import jax
import jax.numpy as jnp
from jax import lax
from jax.experimental import pallas as pl
from jax.experimental.pallas import tpu as pltpu

D = 640
H = 32
DH = 192
F = 1536
EPS = 1e-5
NB = 3
DIST = NB - 1
RT = 16


def _splits(n, k):
    return [(s, min(k, n - s)) for s in range(0, n, k)]


def _kernel(x_hbm, c_hbm, k_hbm, v_hbm, wq_hbm, wo_hbm, wg_hbm, wu_hbm, wd_hbm, wm_hbm,
            o_ref,
            x_v, c_v, wm_v, wq_v, wo_v, wg_v, wu_v, wd_v, kbuf, vbuf, q_scr,
            sem_s, sem_m, sem_q, sem_h, sem_f, sem_d, *, SK, W):
    scale = DH ** -0.5
    f32, bf16 = jnp.float32, jnp.bfloat16
    cnt = [0]

    def start(src, dst, sem):
        pltpu.make_async_copy(src, dst, sem).start(priority=cnt[0] % 2)
        cnt[0] += 1

    def wait(buf, sem):
        pltpu.make_async_copy(buf, buf, sem).wait()

    def start_block(hbm, vm, r0, nr, c0, nc, rch, cch, sem):
        for r in range(r0, r0 + nr, rch):
            for c in range(c0, c0 + nc, cch):
                start(hbm.at[pl.ds(r, rch), pl.ds(c, cch)],
                      vm.at[pl.ds(r, rch), pl.ds(c, cch)], sem)

    kv_cols = _splits(W, 1024)

    def start_head(h, slot):
        for r in range(0, DH, RT):
            for (c0, nc) in kv_cols:
                start(k_hbm.at[h, pl.ds(r, RT), pl.ds(SK - W + c0, nc)],
                      kbuf.at[slot, pl.ds(r, RT), pl.ds(c0, nc)], sem_h.at[slot, 0])
                start(v_hbm.at[h, pl.ds(r, RT), pl.ds(SK - W + c0, nc)],
                      vbuf.at[slot, pl.ds(r, RT), pl.ds(c0, nc)], sem_h.at[slot, 1])
        r0 = h * DH if isinstance(h, int) else pl.multiple_of(h * DH, RT)
        for r in range(0, DH, 32):
            start(wo_hbm.at[pl.ds(r0 + r, 32), :], wo_v.at[pl.ds(r0 + r, 32), :],
                  sem_h.at[slot, 2])
        assert cnt[0] % 2 == 0

    start(c_hbm, c_v, sem_s.at[0])
    start(x_hbm, x_v, sem_s.at[1])
    start_block(wm_hbm, wm_v, 0, D, 0, 1280, RT, 1280, sem_m.at[0])
    NQ = 6
    QG = H * DH // NQ
    for g in range(NQ):
        start_block(wq_hbm, wq_v, 0, D, g * QG, QG, RT, QG, sem_q.at[g])
    start_block(wm_hbm, wm_v, 0, D, 1280, 1280, RT, 1280, sem_m.at[1])
    start_block(wm_hbm, wm_v, 0, D, 2560, 1280, RT, 1280, sem_m.at[2])
    for h in range(DIST):
        start_head(h, h % NB)

    def layernorm(x):
        m = jnp.mean(x, axis=-1, keepdims=True)
        xc = x - m
        v = jnp.mean(xc * xc, axis=-1, keepdims=True)
        return xc / jnp.sqrt(v + EPS)

    wait(c_v, sem_s.at[0])
    cf = jnp.broadcast_to(c_v[...].astype(f32), (8, D))
    sc = (cf * jax.nn.sigmoid(cf)).astype(bf16)
    wait(x_v, sem_s.at[1])
    x0 = jnp.broadcast_to(x_v[...].astype(f32), (8, D))
    ln0 = layernorm(x0)

    wait(wm_v.at[:, pl.ds(0, 1280)], sem_m.at[0])
    mod_a = jnp.dot(sc, wm_v[:, 0:1280], preferred_element_type=f32)
    sa, ca = mod_a[:, 0:D], mod_a[:, D:2 * D]
    h1 = (ln0 * (1.0 + ca) + sa).astype(bf16)

    pend = None
    hq = 0
    for g in range(NQ):
        wait(wq_v.at[:, pl.ds(g * QG, QG)], sem_q.at[g])
        qg = jnp.dot(h1, wq_v[:, g * QG:(g + 1) * QG], preferred_element_type=f32)
        pend = qg if pend is None else jnp.concatenate([pend, qg], axis=1)
        n_full = pend.shape[1] // DH
        n_emit = n_full if g == NQ - 1 else (n_full // 2) * 2
        for i in range(n_emit):
            q_scr[hq + i] = pend[:, i * DH:(i + 1) * DH].astype(bf16)
        hq += n_emit
        pend = pend[:, n_emit * DH:] if n_emit * DH < pend.shape[1] else None
    assert hq == H and pend is None

    wait(wm_v.at[:, pl.ds(1280, 1280)], sem_m.at[1])
    mod_b = jnp.dot(sc, wm_v[:, 1280:2560], preferred_element_type=f32)
    wait(wm_v.at[:, pl.ds(2560, 1280)], sem_m.at[2])
    mod_c = jnp.dot(sc, wm_v[:, 2560:3840], preferred_element_type=f32)
    ga, sb = mod_b[:, 0:D], mod_b[:, D:2 * D]
    cb, gb = mod_c[:, 0:D], mod_c[:, D:2 * D]

    FG = 256
    ND = F // FG

    def start_ffn_up():
        for r in range(0, D, RT):
            for c in range(0, F, 768):
                start(wg_hbm.at[pl.ds(r, RT), pl.ds(c, 768)], wg_v.at[pl.ds(r, RT), pl.ds(c, 768)],
                      sem_f.at[0])
                start(wu_hbm.at[pl.ds(r, RT), pl.ds(c, 768)], wu_v.at[pl.ds(r, RT), pl.ds(c, 768)],
                      sem_f.at[1])

    def start_ffn_down():
        for g in range(ND):
            start_block(wd_hbm, wd_v, g * FG, FG, 0, D, 32, D, sem_d.at[g])

    def head_body(h, acc):
        slot = h % NB
        wait(kbuf.at[slot], sem_h.at[slot, 0])
        wait(vbuf.at[slot], sem_h.at[slot, 1])
        r0 = pl.multiple_of(h * DH, RT)
        wait(wo_v.at[pl.ds(r0, DH), :], sem_h.at[slot, 2])

        nxt = h + DIST

        @pl.when(nxt < H)
        def _():
            start_head(nxt, nxt % NB)

        @pl.when(nxt == H)
        def _():
            start_ffn_up()

        @pl.when(nxt == H + 1)
        def _():
            start_ffn_down()

        s = jnp.dot(q_scr[h], kbuf[slot], preferred_element_type=f32) * scale
        m = jnp.max(s, axis=-1, keepdims=True)
        p = jnp.exp(s - m)
        l = jnp.sum(p, axis=-1, keepdims=True)
        o = lax.dot_general(p.astype(bf16), vbuf[slot], (((1,), (1,)), ((), ())),
                            preferred_element_type=f32)
        o = (o / l).astype(bf16)
        return acc + jnp.dot(o, wo_v[pl.ds(r0, DH), :], preferred_element_type=f32)

    attn = lax.fori_loop(0, H, head_body, jnp.zeros((8, D), f32))

    x1 = x0 + ga * attn
    h2 = (layernorm(x1) * (1.0 + cb) + sb).astype(bf16)
    wait(wg_v, sem_f.at[0])
    g_ = jnp.dot(h2, wg_v[...], preferred_element_type=f32)
    wait(wu_v, sem_f.at[1])
    u_ = jnp.dot(h2, wu_v[...], preferred_element_type=f32)
    hh = (g_ * u_).astype(bf16)
    y = jnp.zeros((8, D), f32)
    for g in range(ND):
        wait(wd_v.at[pl.ds(g * FG, FG), :], sem_d.at[g])
        y = y + jnp.dot(hh[:, g * FG:(g + 1) * FG], wd_v[g * FG:(g + 1) * FG, :],
                        preferred_element_type=f32)
    out = x1 + gb * y
    o_ref[...] = out[0:1, :].astype(o_ref.dtype)


@jax.jit
def pallas_adaLN_cond__sliding_block_cached__glu_gated_bilinear__decode_kernel(
    A_x: jax.Array,
    A_k_cache: jax.Array,
    A_v_cache: jax.Array,
    A_wq: jax.Array,
    A_wo: jax.Array,
    B_x: jax.Array,
    B_w_gate: jax.Array,
    B_w_up: jax.Array,
    B_w_down: jax.Array,
    c: jax.Array,
    w_mod: jax.Array,
):
    del B_x
    SK = A_k_cache.shape[2]
    W = min(4096, max(256, SK // 4))
    kT = jnp.transpose(A_k_cache, (0, 1, 3, 2)).reshape(H, DH, SK)
    vT = jnp.transpose(A_v_cache, (0, 1, 3, 2)).reshape(H, DH, SK)
    x2 = A_x.reshape(1, D)
    bf16 = jnp.bfloat16

    hbm = pl.BlockSpec(memory_space=pl.ANY)
    out = pl.pallas_call(
        functools.partial(_kernel, SK=SK, W=W),
        in_specs=[hbm] * 10,
        out_specs=pl.BlockSpec(memory_space=pltpu.VMEM),
        out_shape=jax.ShapeDtypeStruct((1, D), A_x.dtype),
        scratch_shapes=[
            pltpu.VMEM((1, D), bf16),
            pltpu.VMEM((1, D), bf16),
            pltpu.VMEM((D, 6 * D), bf16),
            pltpu.VMEM((D, H * DH), bf16),
            pltpu.VMEM((H * DH, D), bf16),
            pltpu.VMEM((D, F), bf16),
            pltpu.VMEM((D, F), bf16),
            pltpu.VMEM((F, D), bf16),
            pltpu.VMEM((NB, DH, W), bf16),
            pltpu.VMEM((NB, DH, W), bf16),
            pltpu.VMEM((H, 8, DH), bf16),
            pltpu.SemaphoreType.DMA((2,)),
            pltpu.SemaphoreType.DMA((3,)),
            pltpu.SemaphoreType.DMA((6,)),
            pltpu.SemaphoreType.DMA((NB, 3)),
            pltpu.SemaphoreType.DMA((2,)),
            pltpu.SemaphoreType.DMA((6,)),
        ],
        compiler_params=pltpu.CompilerParams(vmem_limit_bytes=64 * 1024 * 1024),
        name="adaln_attn_glu_decode",
    )(x2, c, kT, vT, A_wq, A_wo, B_w_gate, B_w_up, B_w_down, w_mod)
    return out.reshape(A_x.shape)
```

```python
import functools

import jax
import jax.numpy as jnp
from jax import lax
from jax.experimental import pallas as pl
from jax.experimental.pallas import tpu as pltpu

D = 640
H = 32
DH = 192
F = 1536
EPS = 1e-5
NB = 2
RT = 16
KV_R, KV_C = 32, 512
WQ_R, WQ_C = 16, 1024
WM_R, WM_C = 16, 1280
WG_R, WG_C = 16, 768
WO_R = 32

S_C, S_X = 0, 1
S_M = 2
S_Q = 5
S_F = 11
S_D = 13
S_H = 19
N_SEM = S_H + 3 * NB


def _splits(n, k):
    return [(s, min(k, n - s)) for s in range(0, n, k)]


def _kernel(x_hbm, c_hbm, k_hbm, v_hbm, wq_hbm, wo_hbm, wg_hbm, wu_hbm, wd_hbm, wm_hbm,
            o_ref,
            x_v, c_v, wm_v, wq_v, wo_v, wg_v, wu_v, wd_v, kbuf, vbuf, q_scr, sems, *, SK, W):
    scale = DH ** -0.5
    f32, bf16 = jnp.float32, jnp.bfloat16
    cnt = [0]

    def start(src, dst, sem):
        pltpu.make_async_copy(src, dst, sems.at[sem]).start(priority=cnt[0] % 2)
        cnt[0] += 1

    def wait(buf, sem):
        pltpu.make_async_copy(buf, buf, sems.at[sem]).wait()

    def start_block(hbm, vm, r0, nr, c0, nc, rch, cch, sem):
        for r in range(r0, r0 + nr, rch):
            for c in range(c0, c0 + nc, cch):
                start(hbm.at[pl.ds(r, rch), pl.ds(c, cch)],
                      vm.at[pl.ds(r, rch), pl.ds(c, cch)], sem)

    def start_kv(h, slot, cols):
        for c0 in cols:
            for r in range(0, DH, KV_R):
                start(k_hbm.at[h, pl.ds(r, KV_R), pl.ds(SK - W + c0, KV_C)],
                      kbuf.at[slot, pl.ds(r, KV_R), pl.ds(c0, KV_C)], S_H + 3 * slot)
                start(v_hbm.at[h, pl.ds(r, KV_R), pl.ds(SK - W + c0, KV_C)],
                      vbuf.at[slot, pl.ds(r, KV_R), pl.ds(c0, KV_C)], S_H + 3 * slot + 1)

    def start_wo(h, slot):
        r0 = h * DH if isinstance(h, int) else pl.multiple_of(h * DH, RT)
        for r in range(0, DH, WO_R):
            start(wo_hbm.at[pl.ds(r0 + r, WO_R), :], wo_v.at[pl.ds(r0 + r, WO_R), :],
                  S_H + 3 * slot + 2)

    def start_head(h, slot):
        start_kv(h, slot, range(0, W, KV_C))
        start_wo(h, slot)
        assert cnt[0] % 2 == 0

    def layernorm(x):
        m = jnp.mean(x, axis=-1, keepdims=True)
        xc = x - m
        v = jnp.mean(xc * xc, axis=-1, keepdims=True)
        return xc / jnp.sqrt(v + EPS)

    NQ = 6
    QG = H * DH // NQ

    def start_q(g):
        start_block(wq_hbm, wq_v, 0, D, g * QG, QG, WQ_R, WQ_C, S_Q + g)

    def start_mod(g):
        start_block(wm_hbm, wm_v, 0, D, g * 1280, 1280, WM_R, WM_C, S_M + g)

    def mod_part(g, sc):
        wait(wm_v.at[:, pl.ds(g * 1280, 1280)], S_M + g)
        m = jnp.dot(sc, wm_v[:, g * 1280:(g + 1) * 1280], preferred_element_type=f32)
        return m[:, 0:D], m[:, D:2 * D]

    start(c_hbm, c_v, S_C)
    start(x_hbm, x_v, S_X)
    start_mod(0)
    start_q(0)

    wait(c_v, S_C)
    cf = jnp.broadcast_to(c_v[...].astype(f32), (8, D))
    sc = (cf * jax.nn.sigmoid(cf)).astype(bf16)
    wait(x_v, S_X)
    x0 = jnp.broadcast_to(x_v[...].astype(f32), (8, D))
    ln0 = layernorm(x0)

    start_q(1)
    sa, ca = mod_part(0, sc)
    h1 = (ln0 * (1.0 + ca) + sa).astype(bf16)

    ahead = [lambda: start_q(2), lambda: start_q(3), lambda: start_q(4), lambda: start_q(5),
             lambda: start_mod(1), lambda: start_mod(2)]
    pend = None
    hq = 0
    for g in range(NQ):
        ahead[g]()
        wait(wq_v.at[:, pl.ds(g * QG, QG)], S_Q + g)
        qg = jnp.dot(h1, wq_v[:, g * QG:(g + 1) * QG], preferred_element_type=f32)
        pend = qg if pend is None else jnp.concatenate([pend, qg], axis=1)
        n_full = pend.shape[1] // DH
        n_emit = n_full if g == NQ - 1 else (n_full // 2) * 2
        for i in range(n_emit):
            q_scr[hq + i] = pend[:, i * DH:(i + 1) * DH].astype(bf16)
        hq += n_emit
        pend = pend[:, n_emit * DH:] if n_emit * DH < pend.shape[1] else None
    assert hq == H and pend is None

    start_kv(0, 0, range(0, W // 2, KV_C))
    ga, sb = mod_part(1, sc)
    start_kv(0, 0, range(W // 2, W, KV_C))
    start_wo(0, 0)
    cb, gb = mod_part(2, sc)

    def attend(h, acc):
        slot = h % NB
        r0 = h * DH if isinstance(h, int) else pl.multiple_of(h * DH, RT)
        wait(kbuf.at[slot], S_H + 3 * slot)
        s = jnp.dot(q_scr[h], kbuf[slot], preferred_element_type=f32) * scale
        m = jnp.max(s, axis=-1, keepdims=True)
        p = jnp.exp(s - m)
        l = jnp.sum(p, axis=-1, keepdims=True)
        wait(vbuf.at[slot], S_H + 3 * slot + 1)
        o = lax.dot_general(p.astype(bf16), vbuf[slot], (((1,), (1,)), ((), ())),
                            preferred_element_type=f32)
        o = (o / l).astype(bf16)
        wait(wo_v.at[pl.ds(r0, DH), :], S_H + 3 * slot + 2)
        return acc + jnp.dot(o, wo_v[pl.ds(r0, DH), :], preferred_element_type=f32)

    def head_body(h, acc):
        start_head(h + 1, (h + 1) % NB)
        return attend(h, acc)

    attn = lax.fori_loop(0, H - 1, head_body, jnp.zeros((8, D), f32))

    FG = 256
    ND = F // FG

    def start_ffn_up(rows):
        for r in rows:
            for c in range(0, F, WG_C):
                start(wg_hbm.at[pl.ds(r, WG_R), pl.ds(c, WG_C)],
                      wg_v.at[pl.ds(r, WG_R), pl.ds(c, WG_C)], S_F)
                start(wu_hbm.at[pl.ds(r, WG_R), pl.ds(c, WG_C)],
                      wu_v.at[pl.ds(r, WG_R), pl.ds(c, WG_C)], S_F + 1)

    start_ffn_up(range(0, 256, WG_R))
    attn = attend(H - 1, attn)
    x1 = x0 + ga * attn
    h2 = (layernorm(x1) * (1.0 + cb) + sb).astype(bf16)
    start_ffn_up(range(256, D, WG_R))
    for g in range(ND):
        start_block(wd_hbm, wd_v, g * FG, FG, 0, D, WO_R, D, S_D + g)

    wait(wg_v, S_F)
    g_ = jnp.dot(h2, wg_v[...], preferred_element_type=f32)
    wait(wu_v, S_F + 1)
    u_ = jnp.dot(h2, wu_v[...], preferred_element_type=f32)
    hh = (g_ * u_).astype(bf16)
    y = jnp.zeros((8, D), f32)
    for g in range(ND):
        wait(wd_v.at[pl.ds(g * FG, FG), :], S_D + g)
        y = y + jnp.dot(hh[:, g * FG:(g + 1) * FG], wd_v[g * FG:(g + 1) * FG, :],
                        preferred_element_type=f32)
    out = x1 + gb * y
    o_ref[...] = out[0:1, :].astype(o_ref.dtype)


@jax.jit
def pallas_adaLN_cond__sliding_block_cached__glu_gated_bilinear__decode_kernel(
    A_x: jax.Array,
    A_k_cache: jax.Array,
    A_v_cache: jax.Array,
    A_wq: jax.Array,
    A_wo: jax.Array,
    B_x: jax.Array,
    B_w_gate: jax.Array,
    B_w_up: jax.Array,
    B_w_down: jax.Array,
    c: jax.Array,
    w_mod: jax.Array,
):
    del B_x
    SK = A_k_cache.shape[2]
    W = min(4096, max(256, SK // 4))
    kT = jnp.transpose(A_k_cache, (0, 1, 3, 2)).reshape(H, DH, SK)
    vT = jnp.transpose(A_v_cache, (0, 1, 3, 2)).reshape(H, DH, SK)
    x2 = A_x.reshape(1, D)
    bf16 = jnp.bfloat16

    hbm = pl.BlockSpec(memory_space=pl.ANY)
    out = pl.pallas_call(
        functools.partial(_kernel, SK=SK, W=W),
        in_specs=[hbm] * 10,
        out_specs=pl.BlockSpec(memory_space=pltpu.VMEM),
        out_shape=jax.ShapeDtypeStruct((1, D), A_x.dtype),
        scratch_shapes=[
            pltpu.VMEM((1, D), bf16),
            pltpu.VMEM((1, D), bf16),
            pltpu.VMEM((D, 6 * D), bf16),
            pltpu.VMEM((D, H * DH), bf16),
            pltpu.VMEM((H * DH, D), bf16),
            pltpu.VMEM((D, F), bf16),
            pltpu.VMEM((D, F), bf16),
            pltpu.VMEM((F, D), bf16),
            pltpu.VMEM((NB, DH, W), bf16),
            pltpu.VMEM((NB, DH, W), bf16),
            pltpu.VMEM((H, 8, DH), bf16),
            pltpu.SemaphoreType.DMA((N_SEM,)),
        ],
        compiler_params=pltpu.CompilerParams(vmem_limit_bytes=64 * 1024 * 1024,
                                             disable_bounds_checks=True),
        name="adaln_attn_glu_decode",
    )(x2, c, kT, vT, A_wq, A_wo, B_w_gate, B_w_up, B_w_down, w_mod)
    return out.reshape(A_x.shape)
```

```python
import functools

import jax
import jax.numpy as jnp
from jax import lax
from jax.experimental import pallas as pl
from jax.experimental.pallas import tpu as pltpu

D = 640
H = 32
DH = 192
F = 1536
EPS = 1e-5
NB = 2
RT = 16
KV_R, KV_C = 32, 512
WQ_R, WQ_C = 16, 1024
WM_R, WM_C = 16, 1280
WG_R, WG_C = 16, 768
WO_R = 16
G_Q0 = 0
WD_R = 16

S_C, S_X = 0, 1
S_M = 2
S_Q = 5
S_F = 11
S_D = 13
S_H = 19
N_SEM = S_H + 3 * NB


def _splits(n, k):
    return [(s, min(k, n - s)) for s in range(0, n, k)]


def _kernel(x_hbm, c_hbm, k_hbm, v_hbm, wq_hbm, wo_hbm, wg_hbm, wu_hbm, wd_hbm, wm_hbm,
            o_ref,
            x_v, c_v, wm_v, wq_v, wo_v, wg_v, wu_v, wd_v, kbuf, vbuf, q_scr, sems, *, SK, W):
    scale = DH ** -0.5
    KV_N = (DH // KV_R) * (W // KV_C)
    f32, bf16 = jnp.float32, jnp.bfloat16
    cnt = [0]

    def start(src, dst, sem, queue=None):
        pltpu.make_async_copy(src, dst, sems.at[sem]).start(
            priority=cnt[0] % 2 if queue is None else queue)
        cnt[0] += 1

    def wait(buf, sem):
        pltpu.make_async_copy(buf, buf, sems.at[sem]).wait()

    def start_block(hbm, vm, r0, nr, c0, nc, rch, cch, sem):
        for r in range(r0, r0 + nr, rch):
            for c in range(c0, c0 + nc, cch):
                start(hbm.at[pl.ds(r, rch), pl.ds(c, cch)],
                      vm.at[pl.ds(r, rch), pl.ds(c, cch)], sem)

    def start_head(h, slot, lo=0, hi=KV_N):
        r0 = h * DH if isinstance(h, int) else pl.multiple_of(h * DH, RT)
        n_wo = DH // WO_R
        for i in range(lo, hi):
            c0, r = (i // (DH // KV_R)) * KV_C, (i % (DH // KV_R)) * KV_R
            start(k_hbm.at[h, pl.ds(r, KV_R), pl.ds(SK - W + c0, KV_C)],
                  kbuf.at[slot, pl.ds(r, KV_R), pl.ds(c0, KV_C)], S_H + 3 * slot, 0)
            start(v_hbm.at[h, pl.ds(r, KV_R), pl.ds(SK - W + c0, KV_C)],
                  vbuf.at[slot, pl.ds(r, KV_R), pl.ds(c0, KV_C)], S_H + 3 * slot + 1, 1)
            for j in range(i * n_wo // KV_N, (i + 1) * n_wo // KV_N):
                start(wo_hbm.at[pl.ds(r0 + j * WO_R, WO_R), :],
                      wo_v.at[pl.ds(r0 + j * WO_R, WO_R), :], S_H + 3 * slot + 2, 0)

    def layernorm(x):
        m = jnp.mean(x, axis=-1, keepdims=True)
        xc = x - m
        v = jnp.mean(xc * xc, axis=-1, keepdims=True)
        return xc / jnp.sqrt(v + EPS)

    NQ = 6
    QG = H * DH // NQ

    def start_q(g):
        start_block(wq_hbm, wq_v, 0, D, g * QG, QG, WQ_R, WQ_C, S_Q + g)

    def start_mod(g):
        start_block(wm_hbm, wm_v, 0, D, g * 1280, 1280, WM_R, WM_C, S_M + g)

    def mod_part(g, sc):
        wait(wm_v.at[:, pl.ds(g * 1280, 1280)], S_M + g)
        m = jnp.dot(sc, wm_v[:, g * 1280:(g + 1) * 1280], preferred_element_type=f32)
        return m[:, 0:D], m[:, D:2 * D]

    start(c_hbm, c_v, S_C)
    start(x_hbm, x_v, S_X)
    start_mod(0)
    start_q(0)

    wait(c_v, S_C)
    cf = jnp.broadcast_to(c_v[...].astype(f32), (8, D))
    sc = (cf * jax.nn.sigmoid(cf)).astype(bf16)
    wait(x_v, S_X)
    x0 = jnp.broadcast_to(x_v[...].astype(f32), (8, D))
    ln0 = layernorm(x0)

    start_q(1)
    sa, ca = mod_part(0, sc)
    h1 = (ln0 * (1.0 + ca) + sa).astype(bf16)

    ahead = [lambda: start_q(2), lambda: start_q(3), lambda: start_q(4), lambda: start_q(5),
             lambda: start_mod(1), lambda: start_mod(2)]
    pend = None
    hq = 0
    for g in range(NQ):
        ahead[g]()
        wait(wq_v.at[:, pl.ds(g * QG, QG)], S_Q + g)
        qg = jnp.dot(h1, wq_v[:, g * QG:(g + 1) * QG], preferred_element_type=f32)
        pend = qg if pend is None else jnp.concatenate([pend, qg], axis=1)
        n_full = pend.shape[1] // DH
        n_emit = n_full if g == NQ - 1 else (n_full // 2) * 2
        for i in range(n_emit):
            q_scr[hq + i] = pend[:, i * DH:(i + 1) * DH].astype(bf16)
        hq += n_emit
        pend = pend[:, n_emit * DH:] if n_emit * DH < pend.shape[1] else None
    assert hq == H and pend is None

    start_head(0, 0, 0, KV_N // 2)
    ga, sb = mod_part(1, sc)
    start_head(0, 0, KV_N // 2, KV_N)
    cb, gb = mod_part(2, sc)

    def attend(h, acc):
        slot = h % NB
        r0 = h * DH if isinstance(h, int) else pl.multiple_of(h * DH, RT)
        wait(kbuf.at[slot], S_H + 3 * slot)
        s = jnp.dot(q_scr[h], kbuf[slot], preferred_element_type=f32) * scale
        m = jnp.max(s, axis=-1, keepdims=True)
        p = jnp.exp(s - m)
        l = jnp.sum(p, axis=-1, keepdims=True)
        wait(vbuf.at[slot], S_H + 3 * slot + 1)
        o = lax.dot_general(p.astype(bf16), vbuf[slot], (((1,), (1,)), ((), ())),
                            preferred_element_type=f32)
        o = (o / l).astype(bf16)
        wait(wo_v.at[pl.ds(r0, DH), :], S_H + 3 * slot + 2)
        return acc + jnp.dot(o, wo_v[pl.ds(r0, DH), :], preferred_element_type=f32)

    def head_body(h, acc):
        start_head(h + 1, (h + 1) % NB)
        return attend(h, acc)

    attn = lax.fori_loop(0, H - 1, head_body, jnp.zeros((8, D), f32))

    FG = 256
    ND = F // FG

    def start_ffn_up(rows):
        for r in rows:
            for c in range(0, F, WG_C):
                start(wg_hbm.at[pl.ds(r, WG_R), pl.ds(c, WG_C)],
                      wg_v.at[pl.ds(r, WG_R), pl.ds(c, WG_C)], S_F, 0)
                start(wu_hbm.at[pl.ds(r, WG_R), pl.ds(c, WG_C)],
                      wu_v.at[pl.ds(r, WG_R), pl.ds(c, WG_C)], S_F + 1, 1)

    start_ffn_up(range(0, 256, WG_R))
    attn = attend(H - 1, attn)
    x1 = x0 + ga * attn
    h2 = (layernorm(x1) * (1.0 + cb) + sb).astype(bf16)
    start_ffn_up(range(256, D, WG_R))
    n_down = F // WD_R
    for i in range(n_down):
        r = i * WD_R
        start(wd_hbm.at[pl.ds(r, WD_R), :], wd_v.at[pl.ds(r, WD_R), :], S_D + r // FG,
              0 if i >= n_down - G_Q0 else i % 2)

    wait(wg_v, S_F)
    g_ = jnp.dot(h2, wg_v[...], preferred_element_type=f32)
    wait(wu_v, S_F + 1)
    u_ = jnp.dot(h2, wu_v[...], preferred_element_type=f32)
    hh = (g_ * u_).astype(bf16)
    y = jnp.zeros((8, D), f32)
    for g in range(ND):
        wait(wd_v.at[pl.ds(g * FG, FG), :], S_D + g)
        y = y + jnp.dot(hh[:, g * FG:(g + 1) * FG], wd_v[g * FG:(g + 1) * FG, :],
                        preferred_element_type=f32)
    out = x1 + gb * y
    o_ref[...] = out[0:1, :].astype(o_ref.dtype)


@jax.jit
def pallas_adaLN_cond__sliding_block_cached__glu_gated_bilinear__decode_kernel(
    A_x: jax.Array,
    A_k_cache: jax.Array,
    A_v_cache: jax.Array,
    A_wq: jax.Array,
    A_wo: jax.Array,
    B_x: jax.Array,
    B_w_gate: jax.Array,
    B_w_up: jax.Array,
    B_w_down: jax.Array,
    c: jax.Array,
    w_mod: jax.Array,
):
    del B_x
    SK = A_k_cache.shape[2]
    W = min(4096, max(256, SK // 4))
    kT = jnp.transpose(A_k_cache, (0, 1, 3, 2)).reshape(H, DH, SK)
    vT = jnp.transpose(A_v_cache, (0, 1, 3, 2)).reshape(H, DH, SK)
    x2 = A_x.reshape(1, D)
    bf16 = jnp.bfloat16

    hbm = pl.BlockSpec(memory_space=pl.ANY)
    out = pl.pallas_call(
        functools.partial(_kernel, SK=SK, W=W),
        in_specs=[hbm] * 10,
        out_specs=pl.BlockSpec(memory_space=pltpu.VMEM),
        out_shape=jax.ShapeDtypeStruct((1, D), A_x.dtype),
        scratch_shapes=[
            pltpu.VMEM((1, D), bf16),
            pltpu.VMEM((1, D), bf16),
            pltpu.VMEM((D, 6 * D), bf16),
            pltpu.VMEM((D, H * DH), bf16),
            pltpu.VMEM((H * DH, D), bf16),
            pltpu.VMEM((D, F), bf16),
            pltpu.VMEM((D, F), bf16),
            pltpu.VMEM((F, D), bf16),
            pltpu.VMEM((NB, DH, W), bf16),
            pltpu.VMEM((NB, DH, W), bf16),
            pltpu.VMEM((H, 8, DH), bf16),
            pltpu.SemaphoreType.DMA((N_SEM,)),
        ],
        compiler_params=pltpu.CompilerParams(vmem_limit_bytes=64 * 1024 * 1024,
                                             disable_bounds_checks=False),
        name="adaln_attn_glu_decode",
    )(x2, c, kT, vT, A_wq, A_wo, B_w_gate, B_w_up, B_w_down, w_mod)
    return out.reshape(A_x.shape)
```

```python
import functools

import jax
import jax.numpy as jnp
from jax import lax
from jax.experimental import pallas as pl
from jax.experimental.pallas import tpu as pltpu

D = 640
H = 32
DH = 192
F = 1536
EPS = 1e-5
NB = 2
RT = 16
KV_R, KV_C = 32, 512
PR = 8
WQ_S, WQ_C = 5, 512
WM_S, WM_C = 4, 640
WG_S, WG_C = 5, 512
WO_R = 16
WD_R = 16

S_C, S_X = 0, 1
S_M = 2
S_Q = 5
S_F = 6
S_D = 8
S_H = 14
N_SEM = S_H + 3 * NB


def _kernel(x_hbm, c_hbm, k_hbm, v_hbm, wq_hbm, wo_hbm, wg_hbm, wu_hbm, wd_hbm, wm_hbm,
            o_ref,
            x_v, c_v, wm_v, wq_v, wo_v, wg_v, wu_v, wd_v, kbuf, vbuf, q_scr, sems, *, SK, W):
    scale = DH ** -0.5
    KV_N = (DH // KV_R) * (W // KV_C)
    f32, bf16 = jnp.float32, jnp.bfloat16

    def start(src, dst, sem, queue):
        pltpu.make_async_copy(src, dst, sems.at[sem]).start(priority=queue)

    def wait(buf, sem):
        pltpu.make_async_copy(buf, buf, sems.at[sem]).wait()

    def start_head(h, slot, lo=0, hi=KV_N):
        r0 = h * DH if isinstance(h, int) else pl.multiple_of(h * DH, RT)
        n_wo = DH // WO_R
        for i in range(lo, hi):
            c0, r = (i // (DH // KV_R)) * KV_C, (i % (DH // KV_R)) * KV_R
            start(k_hbm.at[h, pl.ds(r, KV_R), pl.ds(SK - W + c0, KV_C)],
                  kbuf.at[slot, pl.ds(r, KV_R), pl.ds(c0, KV_C)], S_H + 3 * slot, 0)
            start(v_hbm.at[h, pl.ds(r, KV_R), pl.ds(SK - W + c0, KV_C)],
                  vbuf.at[slot, pl.ds(r, KV_R), pl.ds(c0, KV_C)], S_H + 3 * slot + 1, 1)
            for j in range(i * n_wo // KV_N, (i + 1) * n_wo // KV_N):
                start(wo_hbm.at[pl.ds(r0 + j * WO_R, WO_R), :],
                      wo_v.at[pl.ds(r0 + j * WO_R, WO_R), :], S_H + 3 * slot + 2, 0)

    def layernorm(x):
        m = jnp.mean(x, axis=-1, keepdims=True)
        xc = x - m
        v = jnp.mean(xc * xc, axis=-1, keepdims=True)
        return xc / jnp.sqrt(v + EPS)

    def start_halves(hbm, vm, r0, nr, c0, nc, rch, cch, sem, lo=0, hi=None, sem_per_half=False):
        pieces = [(r, c) for r in range(0, nr // 2, rch) for c in range(c0, c0 + nc, cch)]
        for (r, c) in pieces[lo:hi]:
            for q in range(2):
                rr = r0 + r + q * (nr // 2)
                start(hbm.at[pl.ds(rr, rch), pl.ds(c, cch)], vm.at[pl.ds(rr, rch), pl.ds(c, cch)],
                      sem + q if sem_per_half else sem, q)

    def seg_pieces(rows, c0, nc, cch):
        p = [(r, c) for r in range(0, rows, PR) for c in range(c0, c0 + nc, cch)]
        return list(zip(p[:len(p) // 2], p[len(p) // 2:]))

    def start_seg(hbm, vm, pairs, cch, sem):
        for pair in pairs:
            for q, (r, c) in enumerate(pair):
                start(hbm.at[:, pl.ds(r, PR), pl.ds(c, cch)], vm.at[:, pl.ds(r, PR), pl.ds(c, cch)],
                      sem, q)

    def rows2d(ref, c0, nc):
        v = ref[:, :, c0:c0 + nc]
        return v.reshape(v.shape[0] * v.shape[1], nc)

    def start_mod(g):
        start_seg(wm_hbm, wm_v, seg_pieces(D // WM_S, g * 1280, 1280, WM_C), WM_C, S_M + g)

    def mod_part(g, sc):
        wait(wm_v.at[:, :, pl.ds(g * 1280, 1280)], S_M + g)
        m = jnp.dot(sc, rows2d(wm_v, g * 1280, 1280), preferred_element_type=f32)
        return m[:, 0:D], m[:, D:2 * D]

    wq_pairs = seg_pieces(D // WQ_S, 0, H * DH, WQ_C)
    n_wq = len(wq_pairs)
    start(c_hbm, c_v, S_C, 0)
    start(x_hbm, x_v, S_X, 1)
    start_mod(0)
    start_seg(wq_hbm, wq_v, wq_pairs[:n_wq // 4], WQ_C, S_Q)

    wait(c_v, S_C)
    cf = jnp.broadcast_to(c_v[...].astype(f32), (8, D))
    sc = (cf * jax.nn.sigmoid(cf)).astype(bf16)
    wait(x_v, S_X)
    x0 = jnp.broadcast_to(x_v[...].astype(f32), (8, D))
    ln0 = layernorm(x0)

    start_seg(wq_hbm, wq_v, wq_pairs[n_wq // 4:n_wq // 2], WQ_C, S_Q)
    sa, ca = mod_part(0, sc)
    h1 = (ln0 * (1.0 + ca) + sa).astype(bf16)

    start_seg(wq_hbm, wq_v, wq_pairs[n_wq // 2:], WQ_C, S_Q)
    start_mod(1)
    start_mod(2)
    wait(wq_v, S_Q)
    for hp in range(H // 2):
        qp = jnp.dot(h1, rows2d(wq_v, hp * 2 * DH, 2 * DH), preferred_element_type=f32)
        q_scr[2 * hp] = qp[:, :DH].astype(bf16)
        q_scr[2 * hp + 1] = qp[:, DH:].astype(bf16)

    start_head(0, 0, 0, KV_N // 2)
    ga, sb = mod_part(1, sc)
    start_head(0, 0, KV_N // 2, KV_N)
    cb, gb = mod_part(2, sc)

    def attend(h, acc):
        slot = h % NB
        r0 = h * DH if isinstance(h, int) else pl.multiple_of(h * DH, RT)
        wait(kbuf.at[slot], S_H + 3 * slot)
        s = jnp.dot(q_scr[h], kbuf[slot], preferred_element_type=f32) * scale
        m = jnp.max(s, axis=-1, keepdims=True)
        p = jnp.exp(s - m)
        l = jnp.sum(p, axis=-1, keepdims=True)
        wait(vbuf.at[slot], S_H + 3 * slot + 1)
        o = lax.dot_general(p.astype(bf16), vbuf[slot], (((1,), (1,)), ((), ())),
                            preferred_element_type=f32)
        o = (o / l).astype(bf16)
        wait(wo_v.at[pl.ds(r0, DH), :], S_H + 3 * slot + 2)
        return acc + jnp.dot(o, wo_v[pl.ds(r0, DH), :], preferred_element_type=f32)

    def head_body(h, acc):
        start_head(h + 1, (h + 1) % NB)
        return attend(h, acc)

    attn = lax.fori_loop(0, H - 1, head_body, jnp.zeros((8, D), f32))

    FG = 256
    ND = F // 2 // FG

    up_pieces = [(r, c) for r in range(0, D // WG_S, PR) for c in range(0, F, WG_C)]

    def start_ffn_up(pieces):
        for (r, c) in pieces:
            start(wg_hbm.at[:, pl.ds(r, PR), pl.ds(c, WG_C)],
                  wg_v.at[:, pl.ds(r, PR), pl.ds(c, WG_C)], S_F, 0)
            start(wu_hbm.at[:, pl.ds(r, PR), pl.ds(c, WG_C)],
                  wu_v.at[:, pl.ds(r, PR), pl.ds(c, WG_C)], S_F + 1, 1)

    start_ffn_up(up_pieces)
    attn = attend(H - 1, attn)
    x1 = x0 + ga * attn
    h2 = (layernorm(x1) * (1.0 + cb) + sb).astype(bf16)
    n_dn = F // 2 // WD_R
    for g in range(ND):
        start_halves(wd_hbm, wd_v, 0, F, 0, D, WD_R, D, S_D + 2 * g,
                     g * n_dn // ND, (g + 1) * n_dn // ND, sem_per_half=True)

    wait(wg_v, S_F)
    g_ = jnp.dot(h2, rows2d(wg_v, 0, F), preferred_element_type=f32)
    wait(wu_v, S_F + 1)
    u_ = jnp.dot(h2, rows2d(wu_v, 0, F), preferred_element_type=f32)
    hh = (g_ * u_).astype(bf16)
    y = jnp.zeros((8, D), f32)
    for g in range(ND):
        lo, hi = g * FG, F // 2 + g * FG
        wait(wd_v.at[pl.ds(lo, FG), :], S_D + 2 * g)
        wait(wd_v.at[pl.ds(hi, FG), :], S_D + 2 * g + 1)
        y = y + jnp.dot(jnp.concatenate([hh[:, lo:lo + FG], hh[:, hi:hi + FG]], axis=1),
                        jnp.concatenate([wd_v[lo:lo + FG, :], wd_v[hi:hi + FG, :]], axis=0),
                        preferred_element_type=f32)
    out = x1 + gb * y
    o_ref[...] = out[0:1, :].astype(o_ref.dtype)


@jax.jit
def pallas_adaLN_cond__sliding_block_cached__glu_gated_bilinear__decode_kernel(
    A_x: jax.Array,
    A_k_cache: jax.Array,
    A_v_cache: jax.Array,
    A_wq: jax.Array,
    A_wo: jax.Array,
    B_x: jax.Array,
    B_w_gate: jax.Array,
    B_w_up: jax.Array,
    B_w_down: jax.Array,
    c: jax.Array,
    w_mod: jax.Array,
):
    del B_x
    SK = A_k_cache.shape[2]
    W = min(4096, max(256, SK // 4))
    kT = jnp.transpose(A_k_cache, (0, 1, 3, 2)).reshape(H, DH, SK)
    vT = jnp.transpose(A_v_cache, (0, 1, 3, 2)).reshape(H, DH, SK)
    x2 = A_x.reshape(1, D)
    bf16 = jnp.bfloat16

    hbm = pl.BlockSpec(memory_space=pl.ANY)
    out = pl.pallas_call(
        functools.partial(_kernel, SK=SK, W=W),
        in_specs=[hbm] * 10,
        out_specs=pl.BlockSpec(memory_space=pltpu.VMEM),
        out_shape=jax.ShapeDtypeStruct((1, D), A_x.dtype),
        scratch_shapes=[
            pltpu.VMEM((1, D), bf16),
            pltpu.VMEM((1, D), bf16),
            pltpu.VMEM((WM_S, D // WM_S, 6 * D), bf16),
            pltpu.VMEM((WQ_S, D // WQ_S, H * DH), bf16),
            pltpu.VMEM((H * DH, D), bf16),
            pltpu.VMEM((WG_S, D // WG_S, F), bf16),
            pltpu.VMEM((WG_S, D // WG_S, F), bf16),
            pltpu.VMEM((F, D), bf16),
            pltpu.VMEM((NB, DH, W), bf16),
            pltpu.VMEM((NB, DH, W), bf16),
            pltpu.VMEM((H, 8, DH), bf16),
            pltpu.SemaphoreType.DMA((N_SEM,)),
        ],
        compiler_params=pltpu.CompilerParams(vmem_limit_bytes=64 * 1024 * 1024),
        name="adaln_attn_glu_decode",
    )(x2, c, kT, vT, A_wq.reshape(WQ_S, D // WQ_S, H * DH), A_wo,
      B_w_gate.reshape(WG_S, D // WG_S, F), B_w_up.reshape(WG_S, D // WG_S, F), B_w_down,
      w_mod.reshape(WM_S, D // WM_S, 6 * D))
    return out.reshape(A_x.shape)
```
